```python
import os as _os
_os.environ.setdefault("JAX_PLATFORMS", "cpu")
import jax
import jax.numpy as jnp

def _softmax(x, axis=-1):
    return jax.nn.softmax(x, axis=axis)
def _gelu(x):
    return jax.nn.gelu(x, approximate=True)
def _silu(x):
    return jax.nn.silu(x)
def _sigmoid(x):
    return jax.nn.sigmoid(x)
def _layernorm(x, axis=-1, eps=1e-5):
    m = jnp.mean(x, axis=axis, keepdims=True)
    v = jnp.var(x, axis=axis, keepdims=True)
    return (x - m) / jnp.sqrt(v + eps)
def _scatter_add(tgt, idx, src, axis=0):
    return tgt.at[idx].add(src)
def _segment_sum(src, seg, n):
    return jax.ops.segment_sum(src, seg, n)
class _Rng:
    def __init__(self, key):
        self._k = key
    def _next(self):
        self._k, sub = jax.random.split(self._k)
        return sub
    def normal(self, shape):
        return jax.random.normal(self._next(), shape, dtype=jnp.bfloat16)
    def randint(self, lo, hi, shape):
        return jax.random.randint(self._next(), shape, lo, hi, dtype=jnp.int32)
    def uniform(self, shape, lo=0.0, hi=1.0):
        return jax.random.uniform(self._next(), shape, jnp.bfloat16, lo, hi)
    def permutation(self, n):
        return jax.random.permutation(self._next(), n)


kernel_name = 'standalone__channel_attn_cbam__vision'

def setup_inputs():
    _rng = _Rng(jax.random.key(int.from_bytes(__import__("os").urandom(4), "little")))
    _w = (lambda a: (lambda t: t.astype(jnp.bfloat16) if jnp.issubdtype(t.dtype, jnp.floating) else t)(jnp.asarray(a)))
    H = W = 224
    C = 192
    r = max(C // 4, 1)
    return {
        "x": _w((lambda *s: _rng.normal(s) * 0.2)(1, H, W, C) + (lambda *s: _rng.normal(s) * 0.2)(1, 1, 1, C) * 2.0),
        "w1": _w((lambda *s: _rng.normal(s) * 0.2)(C, r)),
        "w2": _w((lambda *s: _rng.normal(s) * 0.2)(r, C)),
    }

def reference(x, w1, w2):
    B, H, W, C = x.shape
    xf = x.reshape(B, H * W, C)
    gap = jnp.mean(xf, 1)
    gmp = jnp.amax(xf, 1)
    h_a = gap @ w1
    h_a = h_a * (lambda x, dt: x.astype(dt))(h_a > 0, h_a.dtype)
    h_m = gmp @ w1
    h_m = h_m * (lambda x, dt: x.astype(dt))(h_m > 0, h_m.dtype)
    scale = _sigmoid(h_a @ w2 + h_m @ w2)
    return x * scale[:, None, None, :]
```

```python
import functools, jax, jax.numpy as jnp
from jax import lax
from jax.experimental import pallas as pl
from jax.experimental.pallas import tpu as pltpu

def make(read_chunks=(8,16,32,32,32,32,32,24,8,4,2,2), look=3, wB=32, first_split=(1,4,16)):
    def fn(x, w1, w2):
        _, H, W, C = x.shape
        R = w1.shape[1]
        G = 64
        NG = C // G
        NP = H * NG
        A = NP // wB
        assert A * wB == NP and sum(read_chunks) == H
        xt = jnp.transpose(x[0], (0, 2, 1)).reshape(A, wB, G, W)
        w1t = w1.T
        starts = [sum(read_chunks[:i]) for i in range(len(read_chunks))]
        nr = len(read_chunks)
        wd = []
        a0 = 0
        for s in first_split:
            wd.append((a0, s, 0)); a0 += s
        assert a0 == A
        for b in range(1, wB): wd.append((0, A, b))

        def kern(x_hbm, w1_hbm, w2_hbm, o_hbm, xbuf, obuf, w1v, w2v, sacc, macc, scl, rsem, wsem, psem):
            xf_hbm = x_hbm.reshape(NP, G, W)
            xf = xbuf.reshape(NP, G, W)
            def rd(i):
                sl = pl.ds(starts[i]*NG, read_chunks[i]*NG)
                return pltpu.make_async_copy(xf_hbm.at[sl], xf.at[sl], rsem.at[i])
            def wr(k):
                a0, na, b = wd[k]
                return pltpu.make_async_copy(obuf.at[pl.ds(a0, na), pl.ds(b, 1)], o_hbm.at[pl.ds(a0, na), pl.ds(b, 1)], wsem.at[k])
            p1 = pltpu.make_async_copy(w1_hbm, w1v, psem.at[0])
            p2 = pltpu.make_async_copy(w2_hbm, w2v, psem.at[1])
            rd(0).start()
            p1.start(); p2.start()
            for i in range(1, min(look, nr)): rd(i).start()
            sacc[...] = jnp.zeros_like(sacc)
            macc[...] = jnp.full_like(macc, -jnp.inf)
            p1.wait(); p2.wait()
            w2t = w2v[...].astype(jnp.float32).T.astype(jnp.bfloat16)
            for i in range(nr):
                rd(i).wait()
                if i + look < nr: rd(i + look).start()
                h0, nh = starts[i], read_chunks[i]
                for g in range(NG):
                    for r in range(0, G, 32):
                        c0 = g*G + r
                        def body(h, carry):
                            s, m = carry
                            v = xf[h*NG + g, r:r+32, :].astype(jnp.float32)
                            return s + v, jnp.maximum(m, v)
                        s, m = lax.fori_loop(h0, h0+nh, body, (sacc[c0:c0+32, :], macc[c0:c0+32, :]), unroll=min(nh, 2))
                        sacc[c0:c0+32, :] = s
                        macc[c0:c0+32, :] = m
            gap = (jnp.sum(sacc[...], axis=1, keepdims=True) / (H*W)).astype(jnp.bfloat16)
            gmp = jnp.max(macc[...], axis=1, keepdims=True).astype(jnp.bfloat16)
            def mlp(g):
                gb = jnp.broadcast_to(g, (C, 128))
                h = jnp.dot(w1v[...], gb, preferred_element_type=jnp.float32).astype(jnp.bfloat16)
                h = h * (h > 0).astype(h.dtype)
                return jnp.dot(w2t, h, preferred_element_type=jnp.float32).astype(jnp.bfloat16)
            o = (mlp(gap).astype(jnp.float32) + mlp(gmp).astype(jnp.float32)).astype(jnp.bfloat16)
            sc = jax.nn.sigmoid(o.astype(jnp.float32)).astype(jnp.bfloat16).astype(jnp.float32)
            scl[...] = sc.reshape(NG, G, 128)
            for k, (a0, na, b) in enumerate(wd):
                def body(a, _):
                    g = lax.rem(a*wB + b, NG)
                    s = scl[g]
                    s2 = jnp.concatenate([s, s[:, :W-128]], axis=1)
                    obuf[a, b] = (xbuf[a, b].astype(jnp.float32) * s2).astype(jnp.bfloat16)
                    return 0
                lax.fori_loop(a0, a0+na, body, 0)
                wr(k).start()
            for k in range(len(wd)): wr(k).wait()

        o = pl.pallas_call(kern,
            out_shape=jax.ShapeDtypeStruct((A, wB, G, W), jnp.bfloat16),
            in_specs=[pl.BlockSpec(memory_space=pltpu.HBM)]*3,
            out_specs=pl.BlockSpec(memory_space=pltpu.HBM),
            scratch_shapes=[pltpu.VMEM((A, wB, G, W), jnp.bfloat16), pltpu.VMEM((A, wB, G, W), jnp.bfloat16),
                            pltpu.VMEM((R, C), jnp.bfloat16), pltpu.VMEM((R, C), jnp.bfloat16),
                            pltpu.VMEM((C, W), jnp.float32), pltpu.VMEM((C, W), jnp.float32),
                            pltpu.VMEM((NG, G, 128), jnp.float32),
                            pltpu.SemaphoreType.DMA((nr,)), pltpu.SemaphoreType.DMA((len(wd),)), pltpu.SemaphoreType.DMA((2,))],
            compiler_params=pltpu.CompilerParams(vmem_limit_bytes=100*1024*1024))(xt, w1t, w2)
        return jnp.transpose(o.reshape(H, C, W), (0, 2, 1))[None]
    return fn


_impl = make()

@jax.jit
def pallas_standalone__channel_attn_cbam__vision_kernel(x, w1, w2):
    return _impl(x, w1, w2)
```

```python
import jax
import jax.numpy as jnp
from jax import lax
import jax.experimental.pallas as pl
import jax.experimental.pallas.tpu as pltpu

F32, BF16 = jnp.float32, jnp.bfloat16

READ_ROWS = (120, 64, 24, 9, 4, 2)
SLAB, PIECE = 2048, 64
HEAD = 16
CBLK = 32


def _round(v):
    return v.astype(BF16).astype(F32)


def _tree_sum(vs):
    while len(vs) > 1:
        vs = [vs[i] + vs[i + 1] if i + 1 < len(vs) else vs[i]
              for i in range(0, len(vs), 2)]
    return vs[0]


@jax.jit
def pallas_standalone__channel_attn_cbam__vision_kernel(
    x: jax.Array,
    w1: jax.Array,
    w2: jax.Array,
):
    B, H, W, C = x.shape
    R = w1.shape[1]
    N = H * C
    NRES = C // PIECE
    NSUP = N // (NRES * SLAB)
    NPIECE = (SLAB - HEAD) // PIECE
    LAST = SLAB - HEAD - NPIECE * PIECE
    SLAB_STEP = (SLAB // PIECE) % NRES
    assert B == 1 and sum(READ_ROWS) == H - 1 and 128 < W <= 256 and R <= 64
    assert NRES * PIECE == C and NSUP * NRES * SLAB == N and LAST > 0
    rows = READ_ROWS + (1,)
    starts = [sum(rows[:i]) for i in range(len(rows))]

    def kernel(x_hbm, w1t_hbm, w2_hbm, o_hbm,
               xbuf, obuf, w1t_v, w2_v, w1d, w2d, sacc, macc, scl,
               rsem, wsem, psem):
        def read(i):
            sl = pl.ds(starts[i] * C, rows[i] * C)
            return pltpu.make_async_copy(x_hbm.at[sl], xbuf.at[sl], rsem.at[i])

        def start_write(*sl):
            pltpu.make_async_copy(obuf.at[sl], o_hbm.at[sl], wsem).start()

        w1_copy = pltpu.make_async_copy(w1t_hbm, w1t_v, psem.at[0])
        w2_copy = pltpu.make_async_copy(w2_hbm, w2_v, psem.at[1])

        def twice_t(w):
            w = w.astype(F32)
            z = jnp.zeros((64 - R, C), F32)
            return jnp.concatenate([w, z, w, z], axis=0).T

        read(0).start()
        w1_copy.start()
        w2_copy.start()
        read(1).start()
        sacc[...] = jnp.zeros((C, W), F32)
        macc[...] = jnp.full((C, W), -jnp.inf, F32)

        for i in range(len(READ_ROWS)):
            read(i).wait()
            if i == 0:
                for j in range(2, len(rows)):
                    read(j).start()
            for c0 in range(0, C, CBLK):
                def accumulate(h, carry, c0=c0):
                    s, m = carry
                    row = pl.multiple_of(h * C + c0, CBLK)
                    v = xbuf[pl.ds(row, CBLK), :].astype(F32)
                    return s + v, jnp.maximum(m, v)

                s, m = lax.fori_loop(
                    starts[i], starts[i] + rows[i], accumulate,
                    (sacc[c0:c0 + CBLK, :], macc[c0:c0 + CBLK, :]),
                    unroll=min(rows[i], 4))
                sacc[c0:c0 + CBLK, :] = s
                macc[c0:c0 + CBLK, :] = m
            if i == 1:
                w1_copy.wait()
                w2_copy.wait()
                w1d[...] = twice_t(w1t_v[...])
                w2t = twice_t(w2_v[...])
                w2d[0:C, :] = w2t
                w2d[C:C + HEAD, :] = w2t[0:HEAD]

        read(len(READ_ROWS)).wait()
        is_avg = lax.broadcasted_iota(jnp.int32, (16, 128), 1) < 64
        parts = []
        for c0 in range(0, C, 16):
            v = xbuf[(H - 1) * C + c0:(H - 1) * C + c0 + 16, :].astype(F32)
            s = sacc[c0:c0 + 16, :] + v
            m = jnp.maximum(macc[c0:c0 + 16, :], v)
            gap = _round(jnp.sum(s, axis=1, keepdims=True) / (H * W))
            gmp = jnp.max(m, axis=1, keepdims=True)
            p = jnp.where(is_avg, gap, gmp) * w1d[c0:c0 + 16, :]
            parts.append(p[:8] + p[8:])
        hid = _round(jnp.sum(_tree_sum(parts), axis=0, keepdims=True))
        hid = hid * (hid > 0).astype(F32)
        lane = lax.broadcasted_iota(jnp.int32, (1, 128), 1)
        h_avg = jnp.where(lane < R, hid, 0.0)
        h_max = jnp.where((lane >= 64) & (lane < 64 + R), hid, 0.0)

        def scale(c0, n):
            w = w2d[pl.ds(c0, n), :]
            o_avg = _round(jnp.sum(w * h_avg, axis=1, keepdims=True))
            o_max = _round(jnp.sum(w * h_max, axis=1, keepdims=True))
            o = jnp.broadcast_to(_round(o_avg + o_max), (n, 128))
            return _round(jax.nn.sigmoid(o))

        def widen(s):
            return jnp.concatenate([s, s[:, :W - 128]], axis=1)

        def gate(a, r, r0, n, s):
            row = pl.multiple_of((a * NRES + r) * SLAB + r0, HEAD)
            v = xbuf[pl.ds(row, n), :].astype(F32)
            obuf[a, r, pl.ds(r0, n), :] = (v * s).astype(BF16)

        def add_mod(t, k):
            return jnp.where(t + k >= NRES, t + k - NRES, t + k)

        for r in range(NRES):
            s = widen(scale((r * SLAB) % C, HEAD))
            for a in range(NSUP):
                gate(a, r, 0, HEAD, s)
            start_write(slice(None), pl.ds(r, 1), pl.ds(0, HEAD))

        def first_piece(r, t):
            c0 = pl.multiple_of(HEAD + PIECE * t, HEAD)
            s = scale(c0, PIECE)
            scl[pl.ds(c0, PIECE), :] = s
            s = widen(s)
            for a in range(NSUP):
                gate(a, r, HEAD, PIECE, s)
            start_write(slice(None), pl.ds(r, 1), pl.ds(HEAD, PIECE))
            return add_mod(t, SLAB_STEP)

        lax.fori_loop(0, NRES, first_piece, jnp.int32(0))

        def piece(b, t, n):
            r0 = pl.multiple_of(HEAD + PIECE * b, HEAD)
            tr = t
            for r in range(NRES):
                c0 = pl.multiple_of(HEAD + PIECE * tr, HEAD)
                s = widen(scl[pl.ds(c0, n), :])

                def slab(a, carry, r=r, s=s):
                    gate(a, r, r0, n, s)
                    return carry

                lax.fori_loop(0, NSUP, slab, 0)
                tr = add_mod(tr, SLAB_STEP)
            start_write(slice(None), slice(None), pl.ds(r0, n))
            return add_mod(t, 1)

        lax.fori_loop(1, NPIECE, lambda b, t: piece(b, t, PIECE), jnp.int32(1))
        piece(NPIECE, jnp.int32(NPIECE % NRES), LAST)
        pltpu.make_async_copy(obuf, o_hbm, wsem).wait()

    hbm = pl.BlockSpec(memory_space=pltpu.HBM)
    out = pl.pallas_call(
        kernel,
        out_shape=jax.ShapeDtypeStruct((NSUP, NRES, SLAB, W), x.dtype),
        in_specs=[hbm, hbm, hbm],
        out_specs=hbm,
        scratch_shapes=[
            pltpu.VMEM((N, W), BF16),
            pltpu.VMEM((NSUP, NRES, SLAB, W), BF16),
            pltpu.VMEM((R, C), BF16),
            pltpu.VMEM((R, C), BF16),
            pltpu.VMEM((C, 128), F32),
            pltpu.VMEM((C + HEAD, 128), F32),
            pltpu.VMEM((C, W), F32),
            pltpu.VMEM((C, W), F32),
            pltpu.VMEM((C + HEAD, 128), F32),
            pltpu.SemaphoreType.DMA((len(rows),)),
            pltpu.SemaphoreType.DMA(()),
            pltpu.SemaphoreType.DMA((2,)),
        ],
        compiler_params=pltpu.CompilerParams(vmem_limit_bytes=64 * 1024 * 1024),
    )(jnp.transpose(x[0], (0, 2, 1)).reshape(N, W), w1.T, w2)
    return jnp.transpose(out.reshape(H, C, W), (0, 2, 1))[None]
```
